```python
import os as _os
_os.environ.setdefault('JAX_PLATFORMS', 'cpu')
import jax
import jax.numpy as jnp

def _softmax(x, axis=-1):
    return jax.nn.softmax(x, axis=axis)

def _gelu(x):
    return jax.nn.gelu(x, approximate=True)

def _silu(x):
    return jax.nn.silu(x)

def _sigmoid(x):
    return jax.nn.sigmoid(x)

def _layernorm(x, axis=-1, eps=1e-05):
    m = jnp.mean(x, axis=axis, keepdims=True)
    v = jnp.var(x, axis=axis, keepdims=True)
    return (x - m) / jnp.sqrt(v + eps)

def _scatter_add(tgt, idx, src, axis=0):
    return tgt.at[idx].add(src)

def _segment_sum(src, seg, n):
    return jax.ops.segment_sum(src, seg, n)

class _Rng:

    def __init__(self, key):
        self._k = key

    def _next(self):
        self._k, sub = jax.random.split(self._k)
        return sub

    def normal(self, shape):
        return jax.random.normal(self._next(), shape, dtype=jnp.bfloat16)

    def randint(self, lo, hi, shape):
        return jax.random.randint(self._next(), shape, lo, hi, dtype=jnp.int32)

    def uniform(self, shape, lo=0.0, hi=1.0):
        return jax.random.uniform(self._next(), shape, jnp.bfloat16, lo, hi)

    def permutation(self, n):
        return jax.random.permutation(self._next(), n)
kernel_name = 'gated_mix__mha_block__memory_aug_recurrent_mem_tr__prompt'

def setup_inputs():
    _rng = _Rng(jax.random.key(int.from_bytes(__import__("os").urandom(4), "little")))
    _w = lambda a: (lambda t: t.astype(jnp.bfloat16) if jnp.issubdtype(t.dtype, jnp.floating) else t)(jnp.asarray(a))

    def _A_setup():
        B, S, D, H = (1, 2048, 512, 32)
        return {'x': _w((lambda *s: _rng.normal(s) * 0.05)(B, S, D)), 'wqkv': _w((lambda *s: _rng.normal(s) * 0.8)(D, 3 * D)), 'wo': _w((lambda *s: _rng.normal(s) * 0.05)(D, D))}
    _A_in = _A_setup()

    def _B_setup():
        B, S, Dm = (1, 2048, 512)
        H, Dh = (32, 128)
        M, seg = (8, 32)
        seg = min(seg, S)
        S = S // seg * seg
        return {'x': _w((lambda *s: _rng.normal(s) * 0.05)(B, S, Dm)), 'mem0': _w((lambda *s: _rng.normal(s) * 0.8)(B, M, Dm)), 'Wq': _w((lambda *s: _rng.normal(s) * 1.6)(Dm, H, Dh) * Dm ** (-0.5)), 'Wk': _w((lambda *s: _rng.normal(s) * 1.6)(Dm, H, Dh) * Dm ** (-0.5)), 'Wv': _w((lambda *s: _rng.normal(s) * 0.8)(Dm, H, Dh) * Dm ** (-0.5)), 'Wo': _w((lambda *s: _rng.normal(s) * 0.8)(H, Dh, Dm) * (H * Dh) ** (-0.5)), 'seg_len': seg}
    _B_in = _B_setup()
    return {'A_x': _A_in['x'], 'A_wqkv': _A_in['wqkv'], 'A_wo': _A_in['wo'], 'B_x': _B_in['x'], 'B_mem0': _B_in['mem0'], 'B_Wq': _B_in['Wq'], 'B_Wk': _B_in['Wk'], 'B_Wv': _B_in['Wv'], 'B_Wo': _B_in['Wo'], 'B_seg_len': _B_in['seg_len'], 'gate_w': _w((lambda *s: _rng.normal(s) * 0.05)(512) * 16.0)}

def reference(A_x, A_wqkv, A_wo, B_x, B_mem0, B_Wq, B_Wk, B_Wv, B_Wo, B_seg_len, gate_w):

    def _A_ref(x, wqkv, wo):
        B, S, D = x.shape
        H = 32
        Dh = D // H
        qkv = (lambda x, *d: x.transpose(*d))((x @ wqkv).reshape(B, S, 3, H, Dh), 2, 0, 3, 1, 4)
        q, k, v = (qkv[0], qkv[1], qkv[2])
        scores = jnp.einsum('bhqd,bhkd->bhqk', q, k) * Dh ** (-0.5)
        p = _softmax(scores, axis=-1)
        o = jnp.einsum('bhqk,bhkd->bhqd', p, v)
        return (lambda x, *d: x.transpose(*d))(o, 0, 2, 1, 3).reshape(B, S, D) @ wo

    def _B_ref(x, mem0, Wq, Wk, Wv, Wo, seg_len):
        B, S, Dm = x.shape
        H, Dh = (Wq.shape[1], Wq.shape[2])
        M = mem0.shape[1]
        scale = Dh ** (-0.5)
        n_seg = S // seg_len
        L = M + seg_len
        idx = jnp.arange(L)
        mask = (idx[:, None] < M) | (idx[:, None] >= idx[None, :])
        mem = mem0
        outs = []
        for s in range(n_seg):
            xs = x[:, s * seg_len:(s + 1) * seg_len, :].copy()
            h = jnp.concatenate([mem, xs], axis=1)
            q = jnp.einsum('btd,dhe->bhte', h, Wq)
            k = jnp.einsum('btd,dhe->bhte', h, Wk)
            v = jnp.einsum('btd,dhe->bhte', h, Wv)
            scores = jnp.einsum('bhqe,bhke->bhqk', q, k) * scale
            scores = jnp.where(mask[None, None], scores, -1000000000.0)
            p = _softmax(scores, axis=-1)
            o = jnp.einsum('bhqk,bhke->bhqe', p, v)
            o = jnp.einsum('bhte,hed->btd', o, Wo)
            mem = o[:, :M, :].copy()
            outs.append(o[:, M:, :])
        return jnp.concatenate(outs, axis=1)
    x = A_x
    g = _sigmoid((x * gate_w).sum(-1, keepdims=True))
    a = _A_ref(x, A_wqkv, A_wo)
    b = _B_ref(x, B_mem0, B_Wq, B_Wk, B_Wv, B_Wo, B_seg_len)
    return g * a + (1 - g) * b
```

```python
import functools

import jax
import jax.numpy as jnp
from jax import lax
import jax.experimental.pallas as pl
import jax.experimental.pallas.tpu as pltpu

F32 = jnp.float32
BF = jnp.bfloat16
U32 = jnp.uint32

LOG2E = 1.4426950408889634

S = 2048
D = 512
HA = 32
DA = 16
HB = 32
DB = 128
MEM = 8
SEG = 32
NSEG = S // SEG
R = SEG + MEM

QT = 256
KC = 256
ACCR = 32
HG = 4
LAGS = (2, 4, 6)
NT = S // QT
SPT = NSEG // NT
UPS = HA // SPT


def _dot(a, b):
    return lax.dot_general(a, b, (((1,), (0,)), ((), ())), preferred_element_type=F32)


def _dot_nt(a, b):
    return lax.dot_general(a, b, (((1,), (1,)), ((), ())), preferred_element_type=F32)


def _interleave(a_items, b_items, wa, wb):
    ta, tb = float(sum(wa)), float(sum(wb))
    out, ia, ib, ca, cb = [], 0, 0, 0.0, 0.0
    while ia < len(a_items) or ib < len(b_items):
        fa = (ca + wa[ia] / 2) / ta if ia < len(a_items) else 2.0
        fb = (cb + wb[ib] / 2) / tb if ib < len(b_items) else 2.0
        if fb <= fa:
            out.append(b_items[ib]); cb += wb[ib]; ib += 1
        else:
            out.append(a_items[ia]); ca += wa[ia]; ia += 1
    return out


def _b_order():
    ng = HB // HG
    la, lb, lo = LAGS
    items = []
    for t in range(ng + max(LAGS)):
        if t < ng:
            items += [("q", t), ("k", t), ("v", t)]
        if 0 <= t - la < ng:
            items.append(("s", t - la))
        if 0 <= t - lb < ng:
            items.append(("p", t - lb))
        if 0 <= t - lo < ng:
            items.append(("o", t - lo))
    return items


def _kernel(x_hbm, wqkv_hbm, woa_hbm, wq_hbm, wk_hbm, wv_hbm, wo_hbm, mem0_ref, gw_ref,
            out_ref,
            x_buf, wqkv_buf, woa_buf, rq, rk, rv, ro, tmp, wq, wk, wv, wo,
            kk, qt, vt, g_buf, s_a, s_b, m_ref, mem_ref, ot_buf, b_buf, sems):
    t = pl.program_id(0)
    NCH = S // KC
    GW = HG * DB

    def qm_of(j):
        h, tt = j % HA, j // HA
        qh = qt[h, :, pl.ds(pl.multiple_of(tt * QT, QT), QT)]
        row = lax.broadcasted_iota(jnp.int32, (64, QT), 0) // 8
        qm = jnp.where(row == (h % 8), jnp.concatenate([qh] * 8, axis=0), jnp.zeros((64, QT), U32))
        return pltpu.bitcast(qm, BF), h // 8

    def qk_chunk(qm, lg, c, s_dst, macc):
        k_tile = pltpu.bitcast(kk[lg, pl.ds(c * KC // 2, KC // 2), :], BF)
        st = _dot(k_tile, qm)
        s_dst[pl.ds(c * KC, KC), :] = st
        mm = jnp.max(st.reshape(KC // ACCR, ACCR, QT), axis=0)
        return mm if macc is None else jnp.maximum(macc, mm)

    def pv_chunk(h, c, s_src, m, lacc, oacc):
        p = jnp.exp2(s_src[pl.ds(c * KC, KC), :] - m)
        ll = jnp.sum(p.reshape(KC // ACCR, ACCR, QT), axis=0)
        v_t = pltpu.bitcast(vt[h, :, pl.ds(c * KC, KC)], BF)
        o_t = _dot(v_t, p.astype(BF))
        return (ll if lacc is None else lacc + ll), (o_t if oacc is None else oacc + o_t)

    @pl.when(t == 0)
    def _prologue():
        pairs = ((x_hbm, x_buf), (wqkv_hbm, wqkv_buf), (wq_hbm, rq), (wk_hbm, rk),
                 (wv_hbm, rv), (wo_hbm, ro), (woa_hbm, woa_buf))
        cps = [pltpu.make_async_copy(a, b, sems.at[i]) for i, (a, b) in enumerate(pairs)]
        for c in cps:
            c.start()
        cps[0].wait()
        cps[1].wait()

        wq_t = jnp.transpose(wqkv_buf[:, 0:D])
        wv_t = jnp.transpose(wqkv_buf[:, 2 * D:3 * D])
        wqv_t = jnp.concatenate([wq_t, wv_t], axis=0)
        gw_rep = jnp.transpose(jnp.broadcast_to(gw_ref[...], (128, D)))
        TC = 512

        def proj(c, carry):
            r0 = pl.multiple_of(c * TC, TC)
            xt = x_buf[pl.ds(r0, TC), :]
            qv = _dot_nt(wqv_t, xt)
            q_t = (qv[:D] * (DA ** -0.5 * LOG2E)).astype(BF)
            v_t = qv[D:].astype(BF)
            qt[:, :, pl.ds(r0, TC)] = pltpu.bitcast(q_t, U32).reshape(HA, 8, TC)
            vt[:, :, pl.ds(r0, TC)] = pltpu.bitcast(v_t, U32).reshape(HA, 8, TC)
            k_n = pltpu.bitcast(_dot(xt, wqkv_buf[:, D:2 * D]).astype(BF), U32)
            r2 = pl.multiple_of(c * (TC // 2), TC // 2)
            for g in range(4):
                kk[g, pl.ds(r2, TC // 2), :] = k_n[:, g * 128:(g + 1) * 128]
            g_buf[pl.ds(r0, TC), :] = jax.nn.sigmoid(_dot(xt, gw_rep))
            return carry

        lax.fori_loop(0, S // TC, proj, 0)

        qm, lg = qm_of(0)
        macc = None
        for c in range(NCH):
            macc = qk_chunk(qm, lg, c, s_a, macc)
        m_ref[...] = jnp.broadcast_to(jnp.max(macc, axis=0, keepdims=True), (8, QT))
        mem_ref[...] = mem0_ref[...].astype(F32)

        for cp, raw, dst in ((cps[2], rq, wq), (cps[3], rk, wk), (cps[4], rv, wv)):
            cp.wait()

            def widen(i, carry, raw=raw):
                tmp[pl.ds(pl.multiple_of(i * 512, 512), 512), :] = pltpu.bitcast(
                    raw[pl.ds(pl.multiple_of(i * 1024, 1024), 1024), :], U32)
                return carry

            lax.fori_loop(0, 16, widen, 0)

            def split(j, carry, dst=dst):
                a = tmp[pl.ds(j, D // 2, stride=32), :]
                b = tmp[pl.ds(j + 16, D // 2, stride=32), :]
                c0 = pl.multiple_of(j * 256, 256)
                dst[:, pl.ds(c0, 128)] = (a & 0xFFFF) | (b << 16)
                dst[:, pl.ds(c0 + 128, 128)] = (a >> 16) | (b & jnp.uint32(0xFFFF0000))
                return carry

            lax.fori_loop(0, 16, split, 0)
        cps[5].wait()

        def pack_o(i, carry):
            wo[pl.ds(pl.multiple_of(i * 128, 128), 128), :] = pltpu.bitcast(
                ro[pl.ds(pl.multiple_of(i * 256, 256), 256), :], U32)
            return carry

        lax.fori_loop(0, 16, pack_o, 0)
        cps[6].wait()

    cb = DB ** -0.5 * LOG2E
    neg = -1e9 * LOG2E

    def step(i, mem):
        s = t * SPT + i
        row = lax.broadcasted_iota(jnp.int32, (R, R), 0)
        col = lax.broadcasted_iota(jnp.int32, (R, R), 1)
        mask = (row >= SEG) | (col >= SEG) | (col <= row)
        xs = x_buf[pl.ds(pl.multiple_of(s * SEG, SEG), SEG), :]
        hb = jnp.concatenate([xs.astype(F32), mem], axis=0)
        bs = dict(q={}, k={}, v={}, p={}, o={}, acc=None)
        ast = {}

        def b_item(kind, g):
            if kind in "qkv":
                w = dict(q=wq, k=wk, v=wv)[kind]
                r = _dot(hb, pltpu.bitcast(w[:, g * GW:(g + 1) * GW], BF))
                bs[kind][g] = r if kind == "q" else r.astype(BF)
            elif kind == "s":
                ps = []
                for j in range(HG):
                    sc = _dot_nt(bs["q"][g][:, j * DB:(j + 1) * DB], bs["k"][g][:, j * DB:(j + 1) * DB])
                    tt = jnp.where(mask, sc * cb, neg)
                    e = jnp.exp2(tt - jnp.max(tt, axis=1, keepdims=True))
                    ps.append(e * (1.0 / jnp.sum(e, axis=1, keepdims=True)))
                bs["p"][g] = ps
            elif kind == "p":
                bs["o"][g] = jnp.concatenate(
                    [_dot(bs["p"][g][j], bs["v"][g][:, j * DB:(j + 1) * DB]) for j in range(HG)], axis=1)
            else:
                z = _dot(bs["o"][g], pltpu.bitcast(wo[g * GW // 2:(g + 1) * GW // 2, :], BF))
                bs["acc"] = z if bs["acc"] is None else bs["acc"] + z

        def a_item(kind, u, c):
            j = t * HA + i * UPS + u
            s_dst, s_src = (s_b, s_a) if u % 2 == 0 else (s_a, s_b)
            if kind == "Q":
                if c == 0:
                    ast["qm"], ast["lg"] = qm_of(jnp.minimum(j + 1, HA * NT - 1))
                    ast["macc"] = None
                ast["macc"] = qk_chunk(ast["qm"], ast["lg"], c, s_dst, ast["macc"])
                if c == NCH - 1:
                    ast["m_next"] = jnp.max(ast["macc"], axis=0, keepdims=True)
            else:
                if c == 0:
                    ast["m"] = m_ref[0:1, :] if u == 0 else ast["m_prev"]
                    ast["lacc"] = ast["oacc"] = None
                h = i * UPS + u
                ast["lacc"], ast["oacc"] = pv_chunk(h, c, s_src, ast["m"], ast["lacc"], ast["oacc"])
                if c == NCH - 1:
                    l = jnp.sum(ast["lacc"], axis=0, keepdims=True)
                    ot_buf[pl.ds(pl.multiple_of(h * DA, DA), DA), :] = ast["oacc"] / l
                    ast["m_prev"] = ast["m_next"]

        a_items = [("a", kind, u, c) for u in range(UPS) for c in range(NCH) for kind in "QV"]
        b_items = [("b",) + it for it in _b_order()]
        wa = [KC * QT / 128 / 4 if it[1] == "Q" else KC / 128 * QT / 128 * 32 / 4 for it in a_items]
        wb = [HG * 10 if it[1] in "sp" else HG * 4 * R / 4 for it in b_items]
        for it in _interleave(a_items, b_items, wa, wb):
            if it[0] == "a":
                a_item(*it[1:])
            else:
                b_item(*it[1:])
        m_ref[...] = jnp.broadcast_to(ast["m_prev"], (8, QT))
        acc = bs["acc"]
        b_buf[pl.ds(pl.multiple_of(i * SEG, SEG), SEG), :] = acc[:SEG]
        return acc[SEG:]

    mem_ref[...] = lax.fori_loop(0, SPT, step, mem_ref[...])

    a = _dot(jnp.transpose(ot_buf[...]), woa_buf[...])
    g = g_buf[pl.ds(pl.multiple_of(t * QT, QT), QT), :]
    g = jnp.concatenate([g] * (D // 128), axis=1)
    out_ref[...] = (g * a + (1.0 - g) * b_buf[...]).astype(out_ref.dtype)


@functools.partial(jax.jit, static_argnames=("B_seg_len",))
def pallas_gated_mix__mha_block__memory_aug_recurrent_mem_tr__prompt_kernel(
    A_x: jax.Array,
    A_wqkv: jax.Array,
    A_wo: jax.Array,
    B_x: jax.Array,
    B_mem0: jax.Array,
    B_Wq: jax.Array,
    B_Wk: jax.Array,
    B_Wv: jax.Array,
    B_Wo: jax.Array,
    B_seg_len: int,
    gate_w: jax.Array,
):
    del B_x
    assert B_seg_len == SEG and A_x.shape == (1, S, D) and B_mem0.shape == (1, MEM, D)
    assert A_wqkv.shape == (D, 3 * D) and B_Wq.shape == (D, HB, DB) and B_Wo.shape == (HB, DB, D)

    any_spec = pl.BlockSpec(memory_space=pl.ANY)
    vm = pltpu.VMEM
    out = pl.pallas_call(
        _kernel,
        grid=(NT,),
        in_specs=[any_spec] * 7 + [
            pl.BlockSpec((MEM, D), lambda t: (0, 0)),
            pl.BlockSpec((1, D), lambda t: (0, 0)),
        ],
        out_specs=pl.BlockSpec((QT, D), lambda t: (t, 0)),
        out_shape=jax.ShapeDtypeStruct((S, D), A_x.dtype),
        scratch_shapes=[
            vm((S, D), BF), vm((D, 3 * D), BF), vm((D, D), BF),
            vm((D * HB, DB), BF), vm((D * HB, DB), BF), vm((D * HB, DB), BF),
            vm((HB * DB, D), BF),
            vm((D * HB // 2, DB), U32),
            vm((D // 2, HB * DB), U32), vm((D // 2, HB * DB), U32), vm((D // 2, HB * DB), U32),
            vm((HB * DB // 2, D), U32),
            vm((4, S // 2, 128), U32), vm((HA, 8, S), U32), vm((HA, 8, S), U32),
            vm((S, 128), F32),
            vm((S, QT), F32), vm((S, QT), F32), vm((8, QT), F32),
            vm((MEM, D), F32), vm((D, QT), F32), vm((QT, D), F32),
            pltpu.SemaphoreType.DMA((7,)),
        ],
        compiler_params=pltpu.CompilerParams(
            dimension_semantics=("arbitrary",), vmem_limit_bytes=100 * 2 ** 20),
        name="gated_mix_fused",
    )(
        A_x.reshape(S, D), A_wqkv, A_wo,
        B_Wq.reshape(D * HB, DB), B_Wk.reshape(D * HB, DB), B_Wv.reshape(D * HB, DB),
        B_Wo.reshape(HB * DB, D), B_mem0.reshape(MEM, D), gate_w.reshape(1, D),
    )
    return out.reshape(1, S, D)
```

```python
import functools

import numpy as np
import jax
import jax.numpy as jnp
from jax import lax
import jax.experimental.pallas as pl
import jax.experimental.pallas.tpu as pltpu

F32 = jnp.float32
BF = jnp.bfloat16
U32 = jnp.uint32

LOG2E = 1.4426950408889634

S = 2048
D = 512
HA, DA = 32, 16
HB, DB = 32, 128
MEM, SEG = 8, 32
NSEG = S // SEG
R = SEG + MEM
RK = R + 8

QT = 256
KC = 128
ACCR = 8
SKEW = 5
HG = 4
LAGS = (2, 3, 4)
BORD = "kvqspo"
UNR = 2
BSPEED, AOFF, VW, TAILW = 1.02, -0.03, 3.0, 50.0
TC = 512
TINY = 2.0 ** -60

NT = S // QT
SPT = NSEG // NT
UPS = HA // SPT
NCH = S // KC
GW = HG * DB


def _dot(a, b):
    return lax.dot_general(a, b, (((1,), (0,)), ((), ())), preferred_element_type=F32)


def _dot_nt(a, b):
    return lax.dot_general(a, b, (((1,), (1,)), ((), ())), preferred_element_type=F32)


def _halves(w):
    return pltpu.bitcast(w << 16, F32), pltpu.bitcast(w & np.uint32(0xFFFF0000), F32)


def _interleave(a_items, b_items, wa, wb):
    ta, tb = float(sum(wa)), float(sum(wb))
    out, ia, ib, ca, cb = [], 0, 0, 0.0, 0.0
    while ia < len(a_items) or ib < len(b_items):
        fa = (ca + wa[ia] / 2) / ta + AOFF if ia < len(a_items) else 2.0
        fb = (cb + wb[ib] / 2) / tb / BSPEED if ib < len(b_items) else 2.0
        if fb <= fa:
            out.append(b_items[ib]); cb += wb[ib]; ib += 1
        else:
            out.append(a_items[ia]); ca += wa[ia]; ia += 1
    return out


def _step_order():
    ng = HB // HG
    lag = dict(q=0, k=0, v=0, s=LAGS[0], p=LAGS[1], o=LAGS[2])
    b_items, wb = [], []
    for u in range(UNR):
        b_items.append(("b", u, "init", 0)); wb.append(0.0)
        for t in range(ng + max(LAGS)):
            for kind in BORD:
                if 0 <= t - lag[kind] < ng:
                    b_items.append(("b", u, kind, t - lag[kind]))
                    wb.append(HG * 10.0 if kind in "sp" else HG * R)
            if t >= ng - 1:
                b_items.append(("b", u, "nop", 0)); wb.append(TAILW)
        b_items.append(("b", u, "fin", 0)); wb.append(0.0)
    chunks = [(uu, c) for uu in range(UNR * UPS) for c in range(NCH)]
    a_items, wa = [], []
    for n in range(len(chunks) + SKEW):
        if n < len(chunks):
            a_items.append(("a", "Q") + chunks[n]); wa.append(KC * QT / 128 / 4)
        if n >= SKEW:
            a_items.append(("a", "V") + chunks[n - SKEW]); wa.append(VW * KC / 128 * QT / 128 * 8)
    return _interleave(a_items, b_items, wa, wb)


def _kernel(x_hbm, wqkv_hbm, woa_hbm, wq_hbm, wk_hbm, wv_hbm, wo_hbm, mem0_ref, gw_ref,
            out_ref,
            x_buf, wqkv_buf, woa_buf, rq, rk, rv, ro, wq, wk, wv, wo,
            kk, qt, vt, g_buf, kb_buf, lmin_ref, s_buf, mem_ref, ot_buf, b_buf, sems):
    t = pl.program_id(0)

    def q_tile(j):
        h, tt = j % HA, j // HA
        qh = qt[h, :, pl.ds(pl.multiple_of(tt * QT, QT), QT)]
        row = lax.broadcasted_iota(jnp.int32, (64, QT), 0) // 8
        qm = jnp.where(row == (h % 8), jnp.concatenate([qh] * 8, axis=0), jnp.zeros((64, QT), U32))
        return pltpu.bitcast(qm, BF), h // 8

    def bound(j):
        h, tt = j % HA, j // HA
        lo, hi = _halves(qt[h, :, pl.ds(pl.multiple_of(tt * QT, QT), QT)])
        q2 = jnp.sum(lo * lo + hi * hi, axis=0, keepdims=True)
        k2 = jnp.concatenate([kb_buf[pl.ds(h, 1), :]] * (QT // 128), axis=1)
        return jnp.sqrt(q2 * k2)

    def k_chunk(lg, c, n):
        return pltpu.bitcast(kk[lg, pl.ds(c * n // 2, n // 2), :], BF)

    def v_chunk(h, c, n):
        return pltpu.bitcast(vt[h, :, pl.ds(c * n, n)], BF)

    cp_x = [pltpu.make_async_copy(x_hbm.at[pl.ds(c * TC, TC)], x_buf.at[pl.ds(c * TC, TC)], sems.at[c])
            for c in range(S // TC)]
    cp_a = [pltpu.make_async_copy(wqkv_hbm.at[:, pl.ds(i * D, D)], wqkv_buf.at[:, pl.ds(i * D, D)], sems.at[4 + i])
            for i in range(3)]
    cp_w = [pltpu.make_async_copy(a, b, sems.at[7 + i])
            for i, (a, b) in enumerate(((wq_hbm, rq), (wk_hbm, rk), (wv_hbm, rv), (wo_hbm, ro)))]
    cp_woa = pltpu.make_async_copy(woa_hbm, woa_buf, sems.at[11])

    @pl.when(t == 0)
    def _prologue():
        for c in [cp_x[0], cp_a[1], cp_a[0], cp_a[2]] + cp_x[1:] + cp_w + [cp_woa]:
            c.start()
        gw_rep = jnp.transpose(jnp.broadcast_to(gw_ref[...].reshape(1, D), (128, D)))
        head_sum = (lax.broadcasted_iota(jnp.int32, (D, 128), 0) // DA
                    == lax.broadcasted_iota(jnp.int32, (D, 128), 1))
        head_sum = jnp.where(head_sum, 1.0, 0.0).astype(BF)

        def k_gate(c, k2max):
            xt = x_buf[pl.ds(c * TC, TC), :]
            k_f = _dot(xt, wqkv_buf[:, D:2 * D])
            k_n = pltpu.bitcast(k_f.astype(BF), U32)
            for g in range(4):
                kk[g, pl.ds(c * TC // 2, TC // 2), :] = k_n[:, g * 128:(g + 1) * 128]
            g_buf[pl.ds(c * TC, TC), :] = jax.nn.sigmoid(_dot(xt, gw_rep))
            n2 = jnp.max(_dot(k_f * k_f, head_sum), axis=0, keepdims=True)
            return n2 if k2max is None else jnp.maximum(k2max, n2)

        def q_v(c, wqv_t):
            xt = x_buf[pl.ds(c * TC, TC), :]
            qv = _dot_nt(wqv_t, xt)
            q_t = (qv[:D] * (DA ** -0.5 * LOG2E)).astype(BF)
            qt[:, :, pl.ds(c * TC, TC)] = pltpu.bitcast(q_t, U32).reshape(HA, 8, TC)
            vt[:, :, pl.ds(c * TC, TC)] = pltpu.bitcast(qv[D:].astype(BF), U32).reshape(HA, 8, TC)

        def relayout(raw, dst):
            nd = 16

            def blk(i, carry):
                v = pltpu.bitcast(raw[pl.ds(pl.multiple_of(i * nd * HB, nd * HB), nd * HB), :], U32)
                v = v.reshape(nd // 8, 8, 2, 8, 128)
                xs = [v[:, a] for a in range(8)]
                sub = lax.broadcasted_iota(jnp.int32, xs[0].shape, 2)
                for sh in (1, 2, 4):
                    keep = (sub & sh) == 0
                    ys = list(xs)
                    for a in range(8):
                        if not a & sh:
                            ys[a] = jnp.where(keep, xs[a], pltpu.roll(xs[a + sh], sh, 2))
                            ys[a + sh] = jnp.where(keep, pltpu.roll(xs[a], 8 - sh, 2), xs[a + sh])
                    xs = ys
                r0 = pl.multiple_of(i * (nd // 2), nd // 2)
                for jl in range(8):
                    for jh in range(2):
                        j = jh * 8 + jl
                        lo, hi = _halves(xs[jl][:, jh].reshape(nd, 128))
                        dst[pl.ds(r0, nd // 2), (2 * j) * 128:(2 * j + 1) * 128] = pltpu.bitcast(lo.astype(BF), U32)
                        dst[pl.ds(r0, nd // 2), (2 * j + 1) * 128:(2 * j + 2) * 128] = pltpu.bitcast(hi.astype(BF), U32)
                return carry

            lax.fori_loop(0, D // nd, blk, 0)

        cp_x[0].wait()
        cp_a[1].wait()
        k2 = k_gate(0, None)
        cp_a[0].wait()
        cp_a[2].wait()
        wqv_t = jnp.concatenate([jnp.transpose(wqkv_buf[:, 0:D]), jnp.transpose(wqkv_buf[:, 2 * D:3 * D])], axis=0)
        q_v(0, wqv_t)
        for c in range(1, S // TC):
            cp_x[c].wait()
            k2 = k_gate(c, k2)
            q_v(c, wqv_t)
            if c < 3:
                cp_w[c - 1].wait()
                relayout((rq, rk)[c - 1], (wq, wk)[c - 1])
        kb_buf[...] = jnp.transpose(jnp.broadcast_to(k2 * (1.0 + 2.0 ** -5), (128, 128)))
        lmin_ref[...] = jnp.ones((8, QT), F32)
        mem_ref[...] = mem0_ref[...].astype(F32)
        cp_w[2].wait()
        relayout(rv, wv)
        cp_w[3].wait()

        def pack_o(i, carry):
            wo[pl.ds(pl.multiple_of(i * 128, 128), 128), :] = pltpu.bitcast(
                ro[pl.ds(pl.multiple_of(i * 256, 256), 256), :], U32)
            return carry

        lax.fori_loop(0, 16, pack_o, 0)

    cb = DB ** -0.5 * LOG2E
    neg = -1e9 * LOG2E

    def body(ib, mem):
        row = lax.broadcasted_iota(jnp.int32, (R, RK), 0)
        col = lax.broadcasted_iota(jnp.int32, (R, RK), 1)
        mask = ((row >= SEG) | (col >= SEG) | (col <= row)) & (col < R)
        st, bs, ast = dict(mem=mem), {}, {}

        def b_item(u, kind, g):
            i = ib * UNR + u
            if kind == "init":
                xs = x_buf[pl.ds(pl.multiple_of((t * SPT + i) * SEG, SEG), SEG), :]
                bs.clear()
                bs.update(q={}, k={}, v={}, p={}, o={}, acc=None)
                bs["hb"] = jnp.concatenate([xs.astype(F32), st["mem"]], axis=0)
            elif kind == "fin":
                b_buf[pl.ds(pl.multiple_of(i * SEG, SEG), SEG), :] = bs["acc"][:SEG]
                st["mem"] = bs["acc"][SEG:]
            elif kind in ("q", "k", "v"):
                w = dict(q=wq, k=wk, v=wv)[kind]
                r = _dot(bs["hb"], pltpu.bitcast(w[:, g * GW:(g + 1) * GW], BF))
                if kind != "q":
                    r = jnp.concatenate([r, jnp.zeros((RK - R, GW), F32)], axis=0).astype(BF)
                bs[kind][g] = r
            elif kind == "s":
                ps = []
                for j in range(HG):
                    sc = _dot_nt(bs["q"][g][:, j * DB:(j + 1) * DB], bs["k"][g][:, j * DB:(j + 1) * DB])
                    tt = jnp.where(mask, sc * cb, neg)
                    e = jnp.exp2(tt - jnp.max(tt, axis=1, keepdims=True))
                    l = jnp.sum(e, axis=1, keepdims=True)
                    r0 = pltpu.reciprocal(l, approx=True)
                    ps.append(e * (r0 * (2.0 - l * r0)))
                bs["p"][g] = ps
            elif kind == "p":
                bs["o"][g] = jnp.concatenate(
                    [_dot(bs["p"][g][j], bs["v"][g][:, j * DB:(j + 1) * DB]) for j in range(HG)], axis=1)
            elif kind == "o":
                z = _dot(bs["o"][g], pltpu.bitcast(wo[g * GW // 2:(g + 1) * GW // 2, :], BF))
                bs["acc"] = z if bs["acc"] is None else bs["acc"] + z

        def a_item(kind, uu, c):
            h = ib * (UNR * UPS) + uu
            j = t * HA + h
            if kind == "Q":
                if c == 0:
                    ast[uu] = q_tile(j) + (bound(j),)
                    ast["l", uu] = None
                qm, lg, mhat = ast[uu]
                p = jnp.exp2(_dot(k_chunk(lg, c, KC), qm) - mhat)
                ll = jnp.sum(p.reshape(KC // ACCR, ACCR, QT), axis=0)
                ast["l", uu] = ll if ast["l", uu] is None else ast["l", uu] + ll
                ast["p", uu, c] = p.astype(BF)
            else:
                o_t = _dot(v_chunk(h, c, KC), ast.pop(("p", uu, c)))
                ast["o"] = o_t if c == 0 else ast["o"] + o_t
                if c == NCH - 1:
                    l = jnp.sum(ast["l", uu], axis=0, keepdims=True)
                    ot_buf[pl.ds(pl.multiple_of(h * DA, DA), DA), :] = ast["o"] / l
                    ast["lmin"] = l if uu == 0 else jnp.minimum(ast["lmin"], l)

        for it in _step_order():
            (a_item if it[0] == "a" else b_item)(*it[1:])
        lmin_ref[...] = jnp.minimum(lmin_ref[...], jnp.broadcast_to(ast["lmin"], (8, QT)))
        return st["mem"]

    mem_ref[...] = lax.fori_loop(0, SPT // UNR, body, mem_ref[...])

    @pl.when(jnp.logical_not(jnp.min(lmin_ref[...]) >= TINY))
    def _exact():
        kc = 256

        def head(h, carry):
            qm, lg = q_tile(t * HA + h)
            m = None
            for c in range(S // kc):
                sc = _dot(k_chunk(lg, c, kc), qm)
                s_buf[pl.ds(c * kc, kc), :] = sc
                mm = jnp.max(sc.reshape(kc // 16, 16, QT), axis=0)
                m = mm if m is None else jnp.maximum(m, mm)
            m = jnp.max(m, axis=0, keepdims=True)
            l = o = None
            for c in range(S // kc):
                p = jnp.exp2(s_buf[pl.ds(c * kc, kc), :] - m)
                ll = jnp.sum(p.reshape(kc // 16, 16, QT), axis=0)
                o_t = _dot(v_chunk(h, c, kc), p.astype(BF))
                l = ll if l is None else l + ll
                o = o_t if o is None else o + o_t
            ot_buf[pl.ds(pl.multiple_of(h * DA, DA), DA), :] = o / jnp.sum(l, axis=0, keepdims=True)
            return carry

        lax.fori_loop(0, HA, head, 0)

    lmin_ref[...] = jnp.ones((8, QT), F32)

    pl.when(t == 0)(cp_woa.wait)
    a = _dot(jnp.transpose(ot_buf[...]), woa_buf[...])
    g = g_buf[pl.ds(pl.multiple_of(t * QT, QT), QT), :]
    g = jnp.concatenate([g] * (D // 128), axis=1)
    out_ref[...] = (g * a + (1.0 - g) * b_buf[...]).astype(out_ref.dtype)


@functools.partial(jax.jit, static_argnames=("B_seg_len",))
def pallas_gated_mix__mha_block__memory_aug_recurrent_mem_tr__prompt_kernel(
    A_x: jax.Array,
    A_wqkv: jax.Array,
    A_wo: jax.Array,
    B_x: jax.Array,
    B_mem0: jax.Array,
    B_Wq: jax.Array,
    B_Wk: jax.Array,
    B_Wv: jax.Array,
    B_Wo: jax.Array,
    B_seg_len: int,
    gate_w: jax.Array,
):
    del B_x
    assert B_seg_len == SEG and A_x.shape == (1, S, D) and B_mem0.shape == (1, MEM, D)
    assert A_wqkv.shape == (D, 3 * D) and A_wo.shape == (D, D) and gate_w.shape == (D,)
    assert B_Wq.shape == B_Wk.shape == B_Wv.shape == (D, HB, DB) and B_Wo.shape == (HB, DB, D)

    any_spec = pl.BlockSpec(memory_space=pl.ANY)
    vm = pltpu.VMEM
    out = pl.pallas_call(
        _kernel,
        grid=(NT,),
        in_specs=[any_spec] * 7 + [
            pl.BlockSpec((MEM, D), lambda t: (0, 0)),
            pl.BlockSpec((D,), lambda t: (0,)),
        ],
        out_specs=pl.BlockSpec((QT, D), lambda t: (t, 0)),
        out_shape=jax.ShapeDtypeStruct((S, D), A_x.dtype),
        scratch_shapes=[
            vm((S, D), BF), vm((D, 3 * D), BF), vm((D, D), BF),
            vm((D * HB, DB), BF), vm((D * HB, DB), BF), vm((D * HB, DB), BF),
            vm((HB * DB, D), BF),
            vm((D // 2, HB * DB), U32), vm((D // 2, HB * DB), U32), vm((D // 2, HB * DB), U32),
            vm((HB * DB // 2, D), U32),
            vm((4, S // 2, 128), U32), vm((HA, 8, S), U32), vm((HA, 8, S), U32),
            vm((S, 128), F32), vm((128, 128), F32), vm((8, QT), F32),
            vm((S, QT), F32),
            vm((MEM, D), F32), vm((D, QT), F32), vm((QT, D), F32),
            pltpu.SemaphoreType.DMA((12,)),
        ],
        compiler_params=pltpu.CompilerParams(
            dimension_semantics=("arbitrary",), vmem_limit_bytes=100 * 2 ** 20),
        name="gated_mix_fused",
    )(
        A_x.reshape(S, D), A_wqkv, A_wo,
        B_Wq.reshape(D * HB, DB), B_Wk.reshape(D * HB, DB), B_Wv.reshape(D * HB, DB),
        B_Wo.reshape(HB * DB, D), B_mem0.reshape(MEM, D), gate_w,
    )
    return out.reshape(1, S, D)
```

```python
import functools

import numpy as np
import jax
import jax.numpy as jnp
from jax import lax
import jax.experimental.pallas as pl
import jax.experimental.pallas.tpu as pltpu

F32 = jnp.float32
BF = jnp.bfloat16
U32 = jnp.uint32

LOG2E = 1.4426950408889634

_reciprocal = pltpu.reciprocal if hasattr(pltpu, "reciprocal") else pl.reciprocal

S = 2048
D = 512
HA, DA = 32, 16
HB, DB = 32, 128
MEM, SEG = 8, 32
NSEG = S // SEG
R = SEG + MEM
RK = R + 8

QT = 256
KC = 128
ACCR = 8
SKEW = 9
HG = 4
LAGS = (1, 5, 6)
BORD = "qkvspo"
UNR = 2
BSPEED, AOFF, VW, TAILW = 1.0, -0.03, 2.0, 150.0
TC = 512
TINY = 2.0 ** -60

NT = S // QT
SPT = NSEG // NT
UPS = HA // SPT
NCH = S // KC
GW = HG * DB


def _dot(a, b):
    return lax.dot_general(a, b, (((1,), (0,)), ((), ())), preferred_element_type=F32)


def _dot_nt(a, b):
    return lax.dot_general(a, b, (((1,), (1,)), ((), ())), preferred_element_type=F32)


def _halves(w):
    return pltpu.bitcast(w << 16, F32), pltpu.bitcast(w & np.uint32(0xFFFF0000), F32)


def _interleave(a_items, b_items, wa, wb):
    ta, tb = float(sum(wa)), float(sum(wb))
    out, ia, ib, ca, cb = [], 0, 0, 0.0, 0.0
    while ia < len(a_items) or ib < len(b_items):
        fa = (ca + wa[ia] / 2) / ta + AOFF if ia < len(a_items) else 2.0
        fb = (cb + wb[ib] / 2) / tb / BSPEED if ib < len(b_items) else 2.0
        if fb <= fa:
            out.append(b_items[ib]); cb += wb[ib]; ib += 1
        else:
            out.append(a_items[ia]); ca += wa[ia]; ia += 1
    return out


def _step_order():
    ng = HB // HG
    lag = dict(q=0, k=0, v=0, s=LAGS[0], p=LAGS[1], o=LAGS[2])
    b_items, wb = [], []
    for u in range(UNR):
        b_items.append(("b", u, "init", 0)); wb.append(0.0)
        for t in range(ng + max(LAGS)):
            for kind in BORD:
                if 0 <= t - lag[kind] < ng:
                    b_items.append(("b", u, kind, t - lag[kind]))
                    wb.append(HG * 10.0 if kind in "sp" else HG * R)
            if t >= ng - 1:
                b_items.append(("b", u, "nop", 0)); wb.append(TAILW)
        b_items.append(("b", u, "fin", 0)); wb.append(0.0)
    chunks = [(uu, c) for uu in range(UNR * UPS) for c in range(NCH)]
    a_items, wa = [], []
    for n in range(len(chunks) + SKEW):
        if n < len(chunks):
            a_items.append(("a", "Q") + chunks[n]); wa.append(KC * QT / 128 / 4)
        if n >= SKEW:
            a_items.append(("a", "V") + chunks[n - SKEW]); wa.append(VW * KC / 128 * QT / 128 * 8)
    return _interleave(a_items, b_items, wa, wb)


def _kernel(x_hbm, wqkv_hbm, woa_hbm, wq_hbm, wk_hbm, wv_hbm, wo_hbm, mem0_hbm, gw_hbm,
            out_ref,
            x_buf, wqkv_buf, woa_buf, rq, rk, rv, wo, wq, wk, wv, kk, qt, vt, g_buf, kb_buf,
            s_buf, ot_buf, b_buf, lmin_ref, mem_ref, mem0_buf, gw_buf, sems):
    t = pl.program_id(0)

    def q_tile(j):
        h, tt = j % HA, j // HA
        qh = qt[h, :, pl.ds(pl.multiple_of(tt * QT, QT), QT)]
        row = lax.broadcasted_iota(jnp.int32, (64, QT), 0) // 8
        qm = jnp.where(row == (h % 8), jnp.concatenate([qh] * 8, axis=0), jnp.zeros((64, QT), U32))
        return pltpu.bitcast(qm, BF), h // 8

    def bound(j):
        h, tt = j % HA, j // HA
        lo, hi = _halves(qt[h, :, pl.ds(pl.multiple_of(tt * QT, QT), QT)])
        q2 = jnp.sum(lo * lo + hi * hi, axis=0, keepdims=True)
        k2 = jnp.concatenate([kb_buf[pl.ds(h, 1), :]] * (QT // 128), axis=1)
        return jnp.sqrt(q2 * k2)

    def k_chunk(lg, c, n):
        return pltpu.bitcast(kk[lg, pl.ds(c * n // 2, n // 2), :], BF)

    def v_chunk(h, c, n):
        return pltpu.bitcast(vt[h, :, pl.ds(c * n, n)], BF)

    cp_x = [pltpu.make_async_copy(x_hbm.at[pl.ds(c * TC, TC)], x_buf.at[pl.ds(c * TC, TC)], sems.at[c])
            for c in range(S // TC)]
    cp_a = [pltpu.make_async_copy(wqkv_hbm.at[:, pl.ds(i * D, D)], wqkv_buf.at[:, pl.ds(i * D, D)], sems.at[4 + i])
            for i in range(3)]
    cp_w = [pltpu.make_async_copy(a, b, sems.at[7 + i])
            for i, (a, b) in enumerate(((wq_hbm, rq), (wk_hbm, rk), (wv_hbm, rv), (wo_hbm, wo)))]
    cp_woa = pltpu.make_async_copy(woa_hbm, woa_buf, sems.at[11])
    cp_gw = pltpu.make_async_copy(gw_hbm, gw_buf, sems.at[12])
    cp_m0 = pltpu.make_async_copy(mem0_hbm, mem0_buf, sems.at[13])

    @pl.when(t == 0)
    def _prologue():
        for c in [cp_x[0], cp_a[1], cp_gw, cp_a[0], cp_a[2], cp_m0] + cp_x[1:] + cp_w + [cp_woa]:
            c.start()
        cp_gw.wait()
        head_sum = (lax.broadcasted_iota(jnp.int32, (D, 128), 0) // DA
                    == lax.broadcasted_iota(jnp.int32, (D, 128), 1))
        head_sum = jnp.where(head_sum, 1.0, 0.0).astype(BF)

        def k_proj(c, k2max):
            xt = x_buf[pl.ds(c * TC, TC), :]
            k_f = _dot(xt, wqkv_buf[:, D:2 * D])
            k_n = pltpu.bitcast(k_f.astype(BF), U32)
            for g in range(4):
                kk[g, pl.ds(c * TC // 2, TC // 2), :] = k_n[:, g * 128:(g + 1) * 128]
            n2 = jnp.max(_dot(k_f * k_f, head_sum), axis=0, keepdims=True)
            return n2 if k2max is None else jnp.maximum(k2max, n2)

        def q_v(c, wqv_t):
            xt = x_buf[pl.ds(c * TC, TC), :]
            qv = _dot_nt(wqv_t, xt)
            q_t = (qv[:D] * (DA ** -0.5 * LOG2E)).astype(BF)
            qt[:, :, pl.ds(c * TC, TC)] = pltpu.bitcast(q_t, U32).reshape(HA, 8, TC)
            vt[:, :, pl.ds(c * TC, TC)] = pltpu.bitcast(qv[D:2 * D].astype(BF), U32).reshape(HA, 8, TC)
            g_buf[:, pl.ds(c * TC, TC)] = jax.nn.sigmoid(qv[2 * D:2 * D + 8])

        def relayout(raw, dst):
            nd = 16

            def blk(i, carry):
                v = pltpu.bitcast(raw[pl.ds(pl.multiple_of(i * nd * HB, nd * HB), nd * HB), :], U32)
                v = v.reshape(nd // 8, 8, 2, 8, 128)
                xs = [v[:, a] for a in range(8)]
                sub = lax.broadcasted_iota(jnp.int32, xs[0].shape, 2)
                for sh in (1, 2, 4):
                    keep = (sub & sh) == 0
                    ys = list(xs)
                    for a in range(8):
                        if not a & sh:
                            ys[a] = jnp.where(keep, xs[a], pltpu.roll(xs[a + sh], sh, 2))
                            ys[a + sh] = jnp.where(keep, pltpu.roll(xs[a], 8 - sh, 2), xs[a + sh])
                    xs = ys
                r0 = pl.multiple_of(i * (nd // 2), nd // 2)
                for jl in range(8):
                    for jh in range(2):
                        j = jh * 8 + jl
                        lo, hi = _halves(xs[jl][:, jh].reshape(nd, 128))
                        dst[pl.ds(r0, nd // 2), (2 * j) * 128:(2 * j + 1) * 128] = pltpu.bitcast(lo.astype(BF), U32)
                        dst[pl.ds(r0, nd // 2), (2 * j + 1) * 128:(2 * j + 2) * 128] = pltpu.bitcast(hi.astype(BF), U32)
                return carry

            lax.fori_loop(0, D // nd, blk, 0)

        cp_x[0].wait()
        cp_a[1].wait()
        k2 = k_proj(0, None)
        cp_a[0].wait()
        cp_a[2].wait()
        wqv_t = jnp.concatenate([jnp.transpose(wqkv_buf[:, 0:D]), jnp.transpose(wqkv_buf[:, 2 * D:3 * D]),
                                 jnp.broadcast_to(gw_buf[...].reshape(1, D), (16, D))], axis=0)
        q_v(0, wqv_t)
        for c in range(1, S // TC):
            cp_x[c].wait()
            k2 = k_proj(c, k2)
            q_v(c, wqv_t)
            if c < 3:
                cp_w[c - 1].wait()
                relayout((rq, rk)[c - 1], (wq, wk)[c - 1])
        kb_buf[...] = jnp.transpose(jnp.broadcast_to(k2 * (1.0 + 2.0 ** -5), (128, 128)))
        lmin_ref[...] = jnp.ones((8, QT), F32)
        cp_m0.wait()
        mem_ref[...] = mem0_buf[...].astype(F32)
        cp_w[2].wait()
        relayout(rv, wv)
        cp_w[3].wait()

    cb = DB ** -0.5 * LOG2E
    neg = -1e9 * LOG2E

    def body(ib, mem):
        row = lax.broadcasted_iota(jnp.int32, (R, RK), 0)
        col = lax.broadcasted_iota(jnp.int32, (R, RK), 1)
        mask = ((row >= SEG) | (col >= SEG) | (col <= row)) & (col < R)
        st, bs, ast = dict(mem=mem), {}, {}

        def b_item(u, kind, g):
            i = ib * UNR + u
            if kind == "init":
                xs = x_buf[pl.ds(pl.multiple_of((t * SPT + i) * SEG, SEG), SEG), :]
                bs.clear()
                bs.update(q={}, k={}, v={}, p={}, o={}, acc=None)
                bs["hb"] = jnp.concatenate([xs.astype(F32), st["mem"]], axis=0)
            elif kind == "fin":
                b_buf[pl.ds(pl.multiple_of(i * SEG, SEG), SEG), :] = bs["acc"][:SEG]
                st["mem"] = bs["acc"][SEG:]
            elif kind in ("q", "k", "v"):
                w = dict(q=wq, k=wk, v=wv)[kind]
                r = _dot(bs["hb"], pltpu.bitcast(w[:, g * GW:(g + 1) * GW], BF))
                if kind != "q":
                    r = jnp.concatenate([r, jnp.zeros((RK - R, GW), F32)], axis=0).astype(BF)
                bs[kind][g] = r
            elif kind == "s":
                ps = []
                for j in range(HG):
                    sc = _dot_nt(bs["q"][g][:, j * DB:(j + 1) * DB], bs["k"][g][:, j * DB:(j + 1) * DB])
                    tt = jnp.where(mask, sc * cb, neg)
                    e = jnp.exp2(tt - jnp.max(tt, axis=1, keepdims=True))
                    l = jnp.sum(e, axis=1, keepdims=True)
                    r0 = _reciprocal(l, approx=True)
                    ps.append(e * (r0 * (2.0 - l * r0)))
                bs["p"][g] = ps
            elif kind == "p":
                bs["o"][g] = jnp.concatenate(
                    [_dot(bs["p"][g][j], bs["v"][g][:, j * DB:(j + 1) * DB]) for j in range(HG)], axis=1)
            elif kind == "o":
                z = _dot(bs["o"][g], wo[g * GW:(g + 1) * GW, :])
                bs["acc"] = z if bs["acc"] is None else bs["acc"] + z

        def a_item(kind, uu, c):
            h = ib * (UNR * UPS) + uu
            j = t * HA + h
            if kind == "Q":
                if c == 0:
                    ast[uu] = q_tile(j) + (bound(j),)
                    ast["l", uu] = None
                qm, lg, mhat = ast[uu]
                p = jnp.exp2(_dot(k_chunk(lg, c, KC), qm) - mhat)
                ll = jnp.sum(p.reshape(KC // ACCR, ACCR, QT), axis=0)
                ast["l", uu] = ll if ast["l", uu] is None else ast["l", uu] + ll
                ast["p", uu, c] = p.astype(BF)
            else:
                o_t = _dot(v_chunk(h, c, KC), ast.pop(("p", uu, c)))
                ast["o"] = o_t if c == 0 else ast["o"] + o_t
                if c == NCH - 1:
                    l = jnp.sum(ast["l", uu], axis=0, keepdims=True)
                    ot_buf[pl.ds(pl.multiple_of(h * DA, DA), DA), :] = ast["o"] / l
                    ast["lmin"] = l if uu == 0 else jnp.minimum(ast["lmin"], l)

        for it in _step_order():
            (a_item if it[0] == "a" else b_item)(*it[1:])
        lmin_ref[...] = jnp.minimum(lmin_ref[...], jnp.broadcast_to(ast["lmin"], (8, QT)))
        return st["mem"]

    mem_ref[...] = lax.fori_loop(0, SPT // UNR, body, mem_ref[...])

    def epilogue():
        a = _dot(jnp.transpose(ot_buf[...]), woa_buf[...])
        g = g_buf[0:1, pl.ds(pl.multiple_of(t * QT, QT), QT)]
        g = jnp.concatenate([jnp.transpose(jnp.broadcast_to(g, (128, QT)))] * (D // 128), axis=1)
        out_ref[...] = (g * a + (1.0 - g) * b_buf[...]).astype(out_ref.dtype)

    def exact():
        kc = 256

        def head(h, carry):
            qm, lg = q_tile(t * HA + h)
            m = None
            for c in range(S // kc):
                sc = _dot(k_chunk(lg, c, kc), qm)
                s_buf[pl.ds(c * kc, kc), :] = sc
                mm = jnp.max(sc.reshape(kc // 16, 16, QT), axis=0)
                m = mm if m is None else jnp.maximum(m, mm)
            m = jnp.max(m, axis=0, keepdims=True)
            l = o = None
            for c in range(S // kc):
                p = jnp.exp2(s_buf[pl.ds(c * kc, kc), :] - m)
                ll = jnp.sum(p.reshape(kc // 16, 16, QT), axis=0)
                o_t = _dot(v_chunk(h, c, kc), p.astype(BF))
                l = ll if l is None else l + ll
                o = o_t if o is None else o + o_t
            ot_buf[pl.ds(pl.multiple_of(h * DA, DA), DA), :] = o / jnp.sum(l, axis=0, keepdims=True)
            return carry

        lax.fori_loop(0, HA, head, 0)

    pl.when(t == 0)(cp_woa.wait)
    unsafe = jnp.logical_not(jnp.min(lmin_ref[...]) >= TINY)
    lmin_ref[...] = jnp.ones((8, QT), F32)
    epilogue()

    @pl.when(unsafe)
    def _():
        exact()
        epilogue()


@functools.partial(jax.jit, static_argnames=("B_seg_len",))
def pallas_gated_mix__mha_block__memory_aug_recurrent_mem_tr__prompt_kernel(
    A_x: jax.Array,
    A_wqkv: jax.Array,
    A_wo: jax.Array,
    B_x: jax.Array,
    B_mem0: jax.Array,
    B_Wq: jax.Array,
    B_Wk: jax.Array,
    B_Wv: jax.Array,
    B_Wo: jax.Array,
    B_seg_len: int,
    gate_w: jax.Array,
):
    del B_x
    assert B_seg_len == SEG and A_x.shape == (1, S, D) and B_mem0.shape == (1, MEM, D)
    assert A_wqkv.shape == (D, 3 * D) and A_wo.shape == (D, D) and gate_w.shape == (D,)
    assert B_Wq.shape == B_Wk.shape == B_Wv.shape == (D, HB, DB) and B_Wo.shape == (HB, DB, D)

    any_spec = pl.BlockSpec(memory_space=pl.ANY)
    vm = pltpu.VMEM
    out = pl.pallas_call(
        _kernel,
        grid=(NT,),
        in_specs=[any_spec] * 9,
        out_specs=pl.BlockSpec((QT, D), lambda t: (t, 0)),
        out_shape=jax.ShapeDtypeStruct((S, D), A_x.dtype),
        scratch_shapes=[
            vm((S, D), BF), vm((D, 3 * D), BF), vm((D, D), BF),
            vm((D * HB, DB), BF), vm((D * HB, DB), BF), vm((D * HB, DB), BF),
            vm((HB * DB, D), BF),
            vm((D // 2, HB * DB), U32), vm((D // 2, HB * DB), U32), vm((D // 2, HB * DB), U32),
            vm((4, S // 2, 128), U32), vm((HA, 8, S), U32), vm((HA, 8, S), U32),
            vm((8, S), F32), vm((128, 128), F32),
            vm((S, QT), F32), vm((D, QT), F32), vm((QT, D), F32),
            vm((8, QT), F32), vm((MEM, D), F32), vm((MEM, D), BF), vm((D,), BF),
            pltpu.SemaphoreType.DMA((14,)),
        ],
        compiler_params=pltpu.CompilerParams(
            dimension_semantics=("arbitrary",), vmem_limit_bytes=64 * 2 ** 20),
        name="gated_mix_fused",
    )(
        A_x.reshape(S, D), A_wqkv, A_wo,
        B_Wq.reshape(D * HB, DB), B_Wk.reshape(D * HB, DB), B_Wv.reshape(D * HB, DB),
        B_Wo.reshape(HB * DB, D), B_mem0.reshape(MEM, D), gate_w,
    )
    return out.reshape(1, S, D)
```
